```python
import os as _os
_os.environ.setdefault('JAX_PLATFORMS', 'cpu')
import jax
import jax.numpy as jnp

def _softmax(x, axis=-1):
    return jax.nn.softmax(x, axis=axis)

def _gelu(x):
    return jax.nn.gelu(x, approximate=True)

def _silu(x):
    return jax.nn.silu(x)

def _sigmoid(x):
    return jax.nn.sigmoid(x)

def _layernorm(x, axis=-1, eps=1e-05):
    m = jnp.mean(x, axis=axis, keepdims=True)
    v = jnp.var(x, axis=axis, keepdims=True)
    return (x - m) / jnp.sqrt(v + eps)

def _scatter_add(tgt, idx, src, axis=0):
    return tgt.at[idx].add(src)

def _segment_sum(src, seg, n):
    return jax.ops.segment_sum(src, seg, n)

class _Rng:

    def __init__(self, key):
        self._k = key

    def _next(self):
        self._k, sub = jax.random.split(self._k)
        return sub

    def normal(self, shape):
        return jax.random.normal(self._next(), shape, dtype=jnp.bfloat16)

    def randint(self, lo, hi, shape):
        return jax.random.randint(self._next(), shape, lo, hi, dtype=jnp.int32)

    def uniform(self, shape, lo=0.0, hi=1.0):
        return jax.random.uniform(self._next(), shape, jnp.bfloat16, lo, hi)

    def permutation(self, n):
        return jax.random.permutation(self._next(), n)
kernel_name = 'adaLN_cond__mha_block_cached__geglu_ffn__prompt'

def setup_inputs():
    _rng = _Rng(jax.random.key(int.from_bytes(__import__("os").urandom(4), "little")))
    _w = lambda a: (lambda t: t.astype(jnp.bfloat16) if jnp.issubdtype(t.dtype, jnp.floating) else t)(jnp.asarray(a))

    def _A_setup():
        B, Sq, D = (1, 2048, 512)
        H, Sk, Dh = (32, 2048, 128)
        return {'x': _w((lambda *s: _rng.normal(s) * 0.05)(B, Sq, D)), 'k_cache': _w((lambda *s: _rng.normal(s) * 3.2)(B, H, Sk, Dh)), 'v_cache': _w((lambda *s: _rng.normal(s) * 0.4)(B, H, Sk, Dh)), 'wq': _w((lambda *s: _rng.normal(s) * 1.6)(D, H * Dh) * D ** (-0.5)), 'wo': _w((lambda *s: _rng.normal(s) * 0.4)(H * Dh, D) * (H * Dh) ** (-0.5))}
    _A_in = _A_setup()

    def _B_setup():
        B, S, D, F = (1, 2048, 512, 1792)
        return {'x': _w((lambda *s: _rng.normal(s) * 0.05)(B, S, D)), 'w_gate': _w((lambda *s: _rng.normal(s) * 0.05)(D, F)), 'w_up': _w((lambda *s: _rng.normal(s) * 0.05)(D, F)), 'w_down': _w((lambda *s: _rng.normal(s) * 0.05)(F, D))}
    _B_in = _B_setup()
    return {'A_x': _A_in['x'], 'A_k_cache': _A_in['k_cache'], 'A_v_cache': _A_in['v_cache'], 'A_wq': _A_in['wq'], 'A_wo': _A_in['wo'], 'B_x': _B_in['x'], 'B_w_gate': _B_in['w_gate'], 'B_w_up': _B_in['w_up'], 'B_w_down': _B_in['w_down'], 'c': _w((lambda *s: _rng.normal(s) * 0.05)(1, 512) * 8.0), 'w_mod': _w((lambda *s: _rng.normal(s) * 0.05)(512, 6 * 512) * 512 ** (-0.5) * 8.0)}

def reference(A_x, A_k_cache, A_v_cache, A_wq, A_wo, B_x, B_w_gate, B_w_up, B_w_down, c, w_mod):

    def _A_ref(x, k_cache, v_cache, wq, wo):
        B, Sq, D = x.shape
        H, Dh = (32, 128)
        q = (lambda x, *d: x.transpose(*d))((x @ wq).reshape(B, Sq, H, Dh), 0, 2, 1, 3)
        scores = jnp.einsum('bhqd,bhkd->bhqk', q, k_cache) * Dh ** (-0.5)
        p = _softmax(scores, axis=-1)
        o = jnp.einsum('bhqk,bhkd->bhqd', p, v_cache)
        return (lambda x, *d: x.transpose(*d))(o, 0, 2, 1, 3).reshape(B, Sq, H * Dh) @ wo

    def _B_ref(x, w_gate, w_up, w_down):
        return _gelu(x @ w_gate) * (x @ w_up) @ w_down
    x = A_x
    mod = (_silu(c) @ w_mod).reshape(c.shape[0], 6, 1, -1)
    sa, ca, ga, sb, cb, gb = (mod[:, 0].copy(), mod[:, 1].copy(), mod[:, 2].copy(), mod[:, 3].copy(), mod[:, 4].copy(), mod[:, 5].copy())
    h = _layernorm(x, axis=-1) * (1 + ca) + sa
    x = x + ga * _A_ref(h, A_k_cache, A_v_cache, A_wq, A_wo)
    h = _layernorm(x, axis=-1) * (1 + cb) + sb
    x = x + gb * _B_ref(h, B_w_gate, B_w_up, B_w_down)
    return x
```

```python
import os
import functools
import math
import jax
import jax.numpy as jnp
from jax import lax
import jax.experimental.pallas as pl
import jax.experimental.pallas.tpu as pltpu

S = 2048
D = 512
H = 32
DH = 128
SK = 2048
F = 1792
EPS = 1e-5
TQ = int(os.environ.get('TQ', 256))
UNROLL = int(os.environ.get('UNROLL', 1))


def _layernorm(x):
    m = jnp.mean(x, axis=-1, keepdims=True)
    xc = x - m
    v = jnp.mean(xc * xc, axis=-1, keepdims=True)
    return xc * lax.rsqrt(v + EPS)


def _gelu_tanh(x):
    c = math.sqrt(2.0 / math.pi)
    return 0.5 * x * (1.0 + jnp.tanh(c * (x + 0.044715 * (x * x * x))))


def kernel(x_ref, k_ref, v_ref, wq_ref, wo_ref, wg_ref, wu_ref, wd_ref, c_ref, wm_ref,
           o_ref, h_scr, acc_scr, mod_scr, q_scr, oh_scr):
    hh = pl.program_id(0)

    @pl.when(hh == 0)
    def _():
        c = c_ref[...].astype(jnp.float32)
        sc = c * jax.nn.sigmoid(c)
        sc8 = jnp.broadcast_to(sc, (8, D)).astype(jnp.bfloat16)
        mod_scr[...] = jnp.dot(sc8, wm_ref[...], preferred_element_type=jnp.float32)
        x = x_ref[...].astype(jnp.float32)
        sa = mod_scr[0:1, 0:D]
        ca = mod_scr[0:1, D:2 * D]
        h_scr[...] = (_layernorm(x) * (1.0 + ca) + sa).astype(jnp.bfloat16)
        acc_scr[...] = jnp.zeros_like(acc_scr)

    scale = DH ** -0.5
    q = jnp.dot(h_scr[...], wq_ref[...], preferred_element_type=jnp.float32)
    q_scr[...] = (q * scale).astype(jnp.bfloat16)
    k = k_ref[...]
    v = v_ref[...]

    def body(j, carry):
        r0 = pl.multiple_of(j * TQ, TQ)
        qs = q_scr[pl.ds(r0, TQ), :]
        s = lax.dot_general(qs, k, (((1,), (1,)), ((), ())), preferred_element_type=jnp.float32)
        m = jnp.max(s, axis=-1, keepdims=True)
        p = jnp.exp(s - m)
        l = jnp.sum(p, axis=-1, keepdims=True)
        o = jnp.dot(p.astype(jnp.bfloat16), v, preferred_element_type=jnp.float32)
        o = o * pl.reciprocal(l, approx=False) if hasattr(pl, 'reciprocal') else o / l
        oh_scr[pl.ds(r0, TQ), :] = o.astype(jnp.bfloat16)
        return carry

    lax.fori_loop(0, S // TQ, body, 0, unroll=UNROLL)
    acc_scr[...] += jnp.dot(oh_scr[...], wo_ref[...], preferred_element_type=jnp.float32)

    @pl.when(hh == H - 1)
    def _():
        x = x_ref[...].astype(jnp.float32)
        ga = mod_scr[0:1, 2 * D:3 * D]
        sb = mod_scr[0:1, 3 * D:4 * D]
        cb = mod_scr[0:1, 4 * D:5 * D]
        gb = mod_scr[0:1, 5 * D:6 * D]
        x1 = x + ga * acc_scr[...]
        h2 = (_layernorm(x1) * (1.0 + cb) + sb).astype(jnp.bfloat16)
        g = jnp.dot(h2, wg_ref[...], preferred_element_type=jnp.float32)
        u = jnp.dot(h2, wu_ref[...], preferred_element_type=jnp.float32)
        a = (_gelu_tanh(g) * u).astype(jnp.bfloat16)
        y = jnp.dot(a, wd_ref[...], preferred_element_type=jnp.float32)
        o_ref[...] = (x1 + gb * y).astype(o_ref.dtype)


@jax.jit
def pallas_adaLN_cond__mha_block_cached__geglu_ffn__prompt_kernel(
    A_x, A_k_cache, A_v_cache, A_wq, A_wo, B_x, B_w_gate, B_w_up, B_w_down, c, w_mod):
    x2 = A_x.reshape(S, D)
    out = pl.pallas_call(
        kernel,
        grid=(H,),
        in_specs=[
            pl.BlockSpec((S, D), lambda h: (0, 0)),
            pl.BlockSpec((None, None, SK, DH), lambda h: (0, h, 0, 0)),
            pl.BlockSpec((None, None, SK, DH), lambda h: (0, h, 0, 0)),
            pl.BlockSpec((D, DH), lambda h: (0, h)),
            pl.BlockSpec((DH, D), lambda h: (h, 0)),
            pl.BlockSpec((D, F), lambda h: (0, 0)),
            pl.BlockSpec((D, F), lambda h: (0, 0)),
            pl.BlockSpec((F, D), lambda h: (0, 0)),
            pl.BlockSpec((1, D), lambda h: (0, 0)),
            pl.BlockSpec((D, 6 * D), lambda h: (0, 0)),
        ],
        out_specs=pl.BlockSpec((S, D), lambda h: (0, 0)),
        out_shape=jax.ShapeDtypeStruct((S, D), jnp.bfloat16),
        scratch_shapes=[
            pltpu.VMEM((S, D), jnp.bfloat16),
            pltpu.VMEM((S, D), jnp.float32),
            pltpu.VMEM((8, 6 * D), jnp.float32),
            pltpu.VMEM((S, DH), jnp.bfloat16),
            pltpu.VMEM((S, DH), jnp.bfloat16),
        ],
        compiler_params=pltpu.CompilerParams(
            dimension_semantics=("arbitrary",),
            vmem_limit_bytes=100 * 1024 * 1024,
        ),
    )(x2, A_k_cache, A_v_cache, A_wq, A_wo, B_w_gate, B_w_up, B_w_down, c, w_mod)
    return out.reshape(1, S, D)
```

```python
import os, math
import jax, jax.numpy as jnp
from jax import lax
import jax.experimental.pallas as pl
import jax.experimental.pallas.tpu as pltpu

S = 2048; D = 512; H = 32; DH = 128; SK = 2048; F = 1792; EPS = 1e-5
TQ = int(os.environ.get('TQ', 256))
TF = int(os.environ.get('TF', 512))

def _layernorm(x):
    m = jnp.mean(x, axis=-1, keepdims=True)
    xc = x - m
    v = jnp.mean(xc * xc, axis=-1, keepdims=True)
    return xc * lax.rsqrt(v + EPS)

def _gelu_tanh(x):
    c = math.sqrt(2.0 / math.pi)
    return 0.5 * x * (1.0 + jnp.tanh(c * (x + 0.044715 * (x * x * x))))

def kernel(x_ref, k_ref, v_ref, wq_ref, wo_ref, wg_hbm, wu_hbm, wd_hbm, c_ref, wm_ref,
           o_ref, h_scr, acc_scr, mod_scr, q_scr, oh_scr, wg_ref, wu_ref, wd_ref, sems):
    hh = pl.program_id(0)

    def w_copies():
        return (pltpu.make_async_copy(wg_hbm, wg_ref, sems.at[0]),
                pltpu.make_async_copy(wu_hbm, wu_ref, sems.at[1]),
                pltpu.make_async_copy(wd_hbm, wd_ref, sems.at[2]))

    @pl.when(hh == 0)
    def _():
        for cp in w_copies():
            cp.start()
        c = c_ref[...].astype(jnp.float32)
        sc = c * jax.nn.sigmoid(c)
        sc8 = jnp.broadcast_to(sc, (8, D)).astype(jnp.bfloat16)
        mod_scr[...] = jnp.dot(sc8, wm_ref[...], preferred_element_type=jnp.float32)
        x = x_ref[...].astype(jnp.float32)
        sa = mod_scr[0:1, 0:D]; ca = mod_scr[0:1, D:2 * D]
        h_scr[...] = (_layernorm(x) * (1.0 + ca) + sa).astype(jnp.bfloat16)
        acc_scr[...] = jnp.zeros_like(acc_scr)

    scale = DH ** -0.5
    q = jnp.dot(h_scr[...], wq_ref[...], preferred_element_type=jnp.float32)
    q_scr[...] = (q * scale).astype(jnp.bfloat16)
    k = k_ref[...]; v = v_ref[...]
    for j in range(S // TQ):
        qs = q_scr[j * TQ:(j + 1) * TQ, :]
        s = lax.dot_general(qs, k, (((1,), (1,)), ((), ())), preferred_element_type=jnp.float32)
        m = jnp.max(s, axis=-1, keepdims=True)
        p = jnp.exp(s - m)
        l = jnp.sum(p, axis=-1, keepdims=True)
        o = jnp.dot(p.astype(jnp.bfloat16), v, preferred_element_type=jnp.float32)
        oh_scr[j * TQ:(j + 1) * TQ, :] = (o / l).astype(jnp.bfloat16)
    acc_scr[...] += jnp.dot(oh_scr[...], wo_ref[...], preferred_element_type=jnp.float32)

    @pl.when(hh == H - 1)
    def _():
        for cp in w_copies():
            cp.wait()
        ga = mod_scr[0:1, 2 * D:3 * D]; sb = mod_scr[0:1, 3 * D:4 * D]
        cb = mod_scr[0:1, 4 * D:5 * D]; gb = mod_scr[0:1, 5 * D:6 * D]
        def ffn_body(j, carry):
            rows = pl.ds(pl.multiple_of(j * TF, TF), TF)
            x1 = x_ref[rows, :].astype(jnp.float32) + ga * acc_scr[rows, :]
            h2 = (_layernorm(x1) * (1.0 + cb) + sb).astype(jnp.bfloat16)
            g = jnp.dot(h2, wg_ref[...], preferred_element_type=jnp.float32)
            u = jnp.dot(h2, wu_ref[...], preferred_element_type=jnp.float32)
            a = (_gelu_tanh(g) * u).astype(jnp.bfloat16)
            y = jnp.dot(a, wd_ref[...], preferred_element_type=jnp.float32)
            o_ref[rows, :] = (x1 + gb * y).astype(o_ref.dtype)
            return carry
        lax.fori_loop(0, S // TF, ffn_body, 0)

@jax.jit
def pallas_adaLN_cond__mha_block_cached__geglu_ffn__prompt_kernel(A_x, A_k_cache, A_v_cache, A_wq, A_wo, B_x, B_w_gate, B_w_up, B_w_down, c, w_mod):
    x2 = A_x.reshape(S, D)
    out = pl.pallas_call(
        kernel, grid=(H,),
        in_specs=[
            pl.BlockSpec((S, D), lambda h: (0, 0)),
            pl.BlockSpec((None, None, SK, DH), lambda h: (0, h, 0, 0)),
            pl.BlockSpec((None, None, SK, DH), lambda h: (0, h, 0, 0)),
            pl.BlockSpec((D, DH), lambda h: (0, h)),
            pl.BlockSpec((DH, D), lambda h: (h, 0)),
            pl.BlockSpec(memory_space=pl.ANY),
            pl.BlockSpec(memory_space=pl.ANY),
            pl.BlockSpec(memory_space=pl.ANY),
            pl.BlockSpec((1, D), lambda h: (0, 0)),
            pl.BlockSpec((D, 6 * D), lambda h: (0, 0)),
        ],
        out_specs=pl.BlockSpec((S, D), lambda h: (0, 0)),
        out_shape=jax.ShapeDtypeStruct((S, D), jnp.bfloat16),
        scratch_shapes=[
            pltpu.VMEM((S, D), jnp.bfloat16), pltpu.VMEM((S, D), jnp.float32),
            pltpu.VMEM((8, 6 * D), jnp.float32), pltpu.VMEM((S, DH), jnp.bfloat16), pltpu.VMEM((S, DH), jnp.bfloat16),
            pltpu.VMEM((D, F), jnp.bfloat16), pltpu.VMEM((D, F), jnp.bfloat16), pltpu.VMEM((F, D), jnp.bfloat16),
            pltpu.SemaphoreType.DMA((3,))],
        compiler_params=pltpu.CompilerParams(dimension_semantics=("arbitrary",), vmem_limit_bytes=100 * 1024 * 1024),
    )(x2, A_k_cache, A_v_cache, A_wq, A_wo, B_w_gate, B_w_up, B_w_down, c, w_mod)
    return out.reshape(1, S, D)
```

```python
import math

import jax
import jax.numpy as jnp
from jax import lax
import jax.experimental.pallas as pl
import jax.experimental.pallas.tpu as pltpu

S = 2048
D = 512
H = 32
DH = 128
SK = 2048
F = 1792
EPS = 1e-5

TQ = 256
TF = 512

QK_SCALE = DH ** -0.5 * math.log2(math.e)


def _layernorm(x):
    m = jnp.mean(x, axis=-1, keepdims=True)
    xc = x - m
    v = jnp.mean(xc * xc, axis=-1, keepdims=True)
    return xc * lax.rsqrt(v + EPS)


def _gelu_tanh(x):
    c = math.sqrt(2.0 / math.pi)
    return 0.5 * x * (1.0 + jnp.tanh(c * (x + 0.044715 * (x * x * x))))


def _silu_rows(c_ref):
    c = c_ref[...].astype(jnp.float32)
    return jnp.broadcast_to(c * jax.nn.sigmoid(c), (8, D)).astype(jnp.bfloat16)


def _kernel(x_ref, k_ref, v_ref, wq_ref, wo_ref, wg_hbm, wu_hbm, wd_hbm, c_ref, wm_ref, wm_hbm,
            o_ref,
            h_scr, acc_scr, mod_scr, q_scr, oh_scr, wg_ref, wu_ref, wd_ref, wm2_ref, sems):
    hh = pl.program_id(0)

    def late_copies():
        return (pltpu.make_async_copy(wg_hbm, wg_ref, sems.at[0]),
                pltpu.make_async_copy(wu_hbm, wu_ref, sems.at[1]),
                pltpu.make_async_copy(wd_hbm, wd_ref, sems.at[2]),
                pltpu.make_async_copy(wm_hbm.at[:, 2 * D:6 * D], wm2_ref, sems.at[3]))

    @pl.when(hh == 0)
    def _():
        for cp in late_copies():
            cp.start()
        mod_scr[:, 0:2 * D] = jnp.dot(_silu_rows(c_ref), wm_ref[...],
                                      preferred_element_type=jnp.float32)
        sa = mod_scr[0:1, 0:D]
        ca = mod_scr[0:1, D:2 * D]
        x = x_ref[...].astype(jnp.float32)
        h_scr[...] = (_layernorm(x) * (1.0 + ca) + sa).astype(jnp.bfloat16)
        acc_scr[...] = jnp.zeros_like(acc_scr)

    q = jnp.dot(h_scr[...], wq_ref[...], preferred_element_type=jnp.float32)
    q_scr[...] = (q * QK_SCALE).astype(jnp.bfloat16)
    k = k_ref[...]
    v = v_ref[...]
    for j in range(S // TQ):
        rows = slice(j * TQ, (j + 1) * TQ)
        s = lax.dot_general(q_scr[rows, :], k, (((1,), (1,)), ((), ())),
                            preferred_element_type=jnp.float32)
        m = jnp.max(s, axis=-1, keepdims=True)
        p = jnp.exp2(s - m)
        l = jnp.sum(p, axis=-1, keepdims=True)
        o = jnp.dot(p.astype(jnp.bfloat16), v, preferred_element_type=jnp.float32)
        oh_scr[rows, :] = (o / l).astype(jnp.bfloat16)
    acc_scr[...] += jnp.dot(oh_scr[...], wo_ref[...], preferred_element_type=jnp.float32)

    @pl.when(hh == H - 1)
    def _():
        for cp in late_copies():
            cp.wait()
        mod_scr[:, 2 * D:6 * D] = jnp.dot(_silu_rows(c_ref), wm2_ref[...],
                                          preferred_element_type=jnp.float32)
        ga = mod_scr[0:1, 2 * D:3 * D]
        sb = mod_scr[0:1, 3 * D:4 * D]
        cb = mod_scr[0:1, 4 * D:5 * D]
        gb = mod_scr[0:1, 5 * D:6 * D]

        def ffn_body(j, carry):
            rows = pl.ds(pl.multiple_of(j * TF, TF), TF)
            x1 = x_ref[rows, :].astype(jnp.float32) + ga * acc_scr[rows, :]
            h2 = (_layernorm(x1) * (1.0 + cb) + sb).astype(jnp.bfloat16)
            g = jnp.dot(h2, wg_ref[...], preferred_element_type=jnp.float32)
            u = jnp.dot(h2, wu_ref[...], preferred_element_type=jnp.float32)
            a = (_gelu_tanh(g) * u).astype(jnp.bfloat16)
            y = jnp.dot(a, wd_ref[...], preferred_element_type=jnp.float32)
            o_ref[rows, :] = (x1 + gb * y).astype(o_ref.dtype)
            return carry

        lax.fori_loop(0, S // TF, ffn_body, 0)


@jax.jit
def pallas_adaLN_cond__mha_block_cached__geglu_ffn__prompt_kernel(
    A_x: jax.Array,
    A_k_cache: jax.Array,
    A_v_cache: jax.Array,
    A_wq: jax.Array,
    A_wo: jax.Array,
    B_x: jax.Array,
    B_w_gate: jax.Array,
    B_w_up: jax.Array,
    B_w_down: jax.Array,
    c: jax.Array,
    w_mod: jax.Array,
):
    x2 = A_x.reshape(S, D)
    out = pl.pallas_call(
        _kernel,
        grid=(H,),
        in_specs=[
            pl.BlockSpec((S, D), lambda h: (0, 0)),
            pl.BlockSpec((None, None, SK, DH), lambda h: (0, h, 0, 0)),
            pl.BlockSpec((None, None, SK, DH), lambda h: (0, h, 0, 0)),
            pl.BlockSpec((D, DH), lambda h: (0, h)),
            pl.BlockSpec((DH, D), lambda h: (h, 0)),
            pl.BlockSpec(memory_space=pl.ANY),
            pl.BlockSpec(memory_space=pl.ANY),
            pl.BlockSpec(memory_space=pl.ANY),
            pl.BlockSpec((1, D), lambda h: (0, 0)),
            pl.BlockSpec((D, 2 * D), lambda h: (0, 0)),
            pl.BlockSpec(memory_space=pl.ANY),
        ],
        out_specs=pl.BlockSpec((S, D), lambda h: (0, 0)),
        out_shape=jax.ShapeDtypeStruct((S, D), jnp.bfloat16),
        scratch_shapes=[
            pltpu.VMEM((S, D), jnp.bfloat16),
            pltpu.VMEM((S, D), jnp.float32),
            pltpu.VMEM((8, 6 * D), jnp.float32),
            pltpu.VMEM((S, DH), jnp.bfloat16),
            pltpu.VMEM((S, DH), jnp.bfloat16),
            pltpu.VMEM((D, F), jnp.bfloat16),
            pltpu.VMEM((D, F), jnp.bfloat16),
            pltpu.VMEM((F, D), jnp.bfloat16),
            pltpu.VMEM((D, 4 * D), jnp.bfloat16),
            pltpu.SemaphoreType.DMA((4,)),
        ],
        compiler_params=pltpu.CompilerParams(
            dimension_semantics=("arbitrary",),
            vmem_limit_bytes=100 * 1024 * 1024,
        ),
    )(x2, A_k_cache, A_v_cache, A_wq, A_wo, B_w_gate, B_w_up, B_w_down, c, w_mod, w_mod)
    return out.reshape(1, S, D)
```
